```python
import jax
import jax.numpy as jnp

def _softmax(x, axis=-1):
    return jax.nn.softmax(x, axis=axis)
def _gelu(x):
    return jax.nn.gelu(x, approximate=True)
def _silu(x):
    return jax.nn.silu(x)
def _sigmoid(x):
    return jax.nn.sigmoid(x)
def _layernorm(x, axis=-1, eps=1e-5):
    m = jnp.mean(x, axis=axis, keepdims=True)
    v = jnp.var(x, axis=axis, keepdims=True)
    return (x - m) / jnp.sqrt(v + eps)
def _scatter_add(tgt, idx, src, axis=0):
    return tgt.at[idx].add(src)
def _segment_sum(src, seg, n):
    return jax.ops.segment_sum(src, seg, n)
class _Rng:
    def __init__(self, key):
        self._k = key
    def _next(self):
        self._k, sub = jax.random.split(self._k)
        return sub
    def normal(self, shape):
        return jax.random.normal(self._next(), shape, dtype=jnp.bfloat16)
    def randint(self, lo, hi, shape):
        return jax.random.randint(self._next(), shape, lo, hi, dtype=jnp.int32)
    def uniform(self, shape, lo=0.0, hi=1.0):
        return jax.random.uniform(self._next(), shape, jnp.bfloat16, lo, hi)
    def permutation(self, n):
        return jax.random.permutation(self._next(), n)


kernel_name = 'gated_mix__sliding_local_dilated__compressed_kv_cla__prompt'

def setup_inputs():
    _rng = _Rng(jax.random.key(int.from_bytes(__import__("os").urandom(4), "little")))
    _w = (lambda a: (lambda t: t.astype(jnp.bfloat16) if jnp.issubdtype(t.dtype, jnp.floating) else t)(jnp.asarray(a)))
    def _A_setup():
        B, S, D = 1, 2048, 576
        return {
            "x": _w((lambda *s: _rng.normal(s) * 0.05)(B, S, D)),
            "wqkv": _w((lambda *s: _rng.normal(s) * 0.05)(D, 3 * D)),
            "wo": _w((lambda *s: _rng.normal(s) * 0.05)(D, D)),
        }
    _A_in = _A_setup()

    def _B_setup():
        B, H, Sq, Sk, D, M = 1, 32, 2048, 2048, 128, 576
        Dc = 4 * D
        return {
            "x": _w((lambda *s: _rng.normal(s) * 0.05)(B, Sq, M)),
            "c_kv": _w((lambda *s: _rng.normal(s) * 0.05)(B, Sk, Dc)),
            "w_q": _w((lambda *s: _rng.normal(s) * 0.05)(M, H, D) * (M ** -0.5)),
            "w_uk": _w((lambda *s: _rng.normal(s) * 0.05)(Dc, H, D) * (Dc ** -0.5)),
            "w_uv": _w((lambda *s: _rng.normal(s) * 0.05)(Dc, H, D) * (Dc ** -0.5)),
            "w_o": _w((lambda *s: _rng.normal(s) * 0.05)(H, D, M) * ((H * D) ** -0.5)),
        }
    _B_in = _B_setup()

    return {
        "A_x": _A_in["x"],
        "A_wqkv": _A_in["wqkv"],
        "A_wo": _A_in["wo"],
        "B_x": _B_in["x"],
        "B_c_kv": _B_in["c_kv"],
        "B_w_q": _B_in["w_q"],
        "B_w_uk": _B_in["w_uk"],
        "B_w_uv": _B_in["w_uv"],
        "B_w_o": _B_in["w_o"],
        "gate_w": _w((lambda *s: _rng.normal(s) * 0.05)(576)),
    }

def reference(A_x, A_wqkv, A_wo, B_x, B_c_kv, B_w_q, B_w_uk, B_w_uv, B_w_o, gate_w):
    def _A_ref(x, wqkv, wo):
        B, S, D = x.shape
        H = 32; Dh = D // H
        W, dil = 8, 2
        qkv = (lambda x, *d: x.transpose(*d))((x @ wqkv).reshape(B, S, 3, H, Dh), 2, 0, 3, 1, 4)
        q, k, v = qkv[0], qkv[1], qkv[2]
        scale = Dh ** -0.5
        pos = jnp.arange(S)
        off = jnp.arange(W) * dil
        idx = pos[:, None] - off[None, :]
        mask = idx >= 0
        idx_c = jnp.where(mask, idx, 0).reshape(-1)
        kg = k[:, :, idx_c, :].reshape(B, H, S, W, Dh)
        vg = v[:, :, idx_c, :].reshape(B, H, S, W, Dh)
        logits = jnp.einsum("bhsd,bhswd->bhsw", q, kg) * scale
        logits = jnp.where(mask[None, None, :, :], logits, -1e9)
        attn = _softmax(logits, axis=-1)
        o = jnp.einsum("bhsw,bhswd->bhsd", attn, vg)
        return (lambda x, *d: x.transpose(*d))(o, 0, 2, 1, 3).reshape(B, S, D) @ wo

    def _B_ref(x, c_kv, w_q, w_uk, w_uv, w_o):
        B, Sq, M = x.shape[0], x.shape[1], x.shape[2]
        Sk = c_kv.shape[1]
        H, D = w_q.shape[1], w_q.shape[2]
        q = jnp.einsum("bqm,mhd->bhqd", x, w_q)
        k = jnp.einsum("bkc,chd->bhkd", c_kv, w_uk)
        v = jnp.einsum("bkc,chd->bhkd", c_kv, w_uv)
        scores = jnp.einsum("bhqd,bhkd->bhqk", q, k) * (D ** -0.5)
        off = Sk - Sq
        qi = jnp.arange(Sq)[:, None]
        kj = jnp.arange(Sk)[None, :]
        cmask = kj <= (qi + off)
        scores = jnp.where(cmask[None, None], scores, -1e9)
        p = _softmax(scores, axis=-1)
        ctx = jnp.einsum("bhqk,bhkd->bhqd", p, v)
        return jnp.einsum("bhqd,hdm->bqm", ctx, w_o)

    x = A_x
    g = _sigmoid((x * gate_w).sum(-1, keepdims=True))
    a = _A_ref(x, A_wqkv, A_wo)
    b = _B_ref(x, B_c_kv, B_w_q, B_w_uk, B_w_uv, B_w_o)
    return g * a + (1 - g) * b
```

```python
import functools
import numpy as np
import jax
import jax.numpy as jnp
from jax import lax
import jax.experimental.pallas as pl
import jax.experimental.pallas.tpu as pltpu

S = 2048
M = 576
H = 32
D = 128
DC = 512
DH = 18
W = 8
DIL = 2
MP = 640
BQ = 256
LOG2E = 1.4426950408889634
F32 = jnp.float32
BF16 = jnp.bfloat16
NT = (((1,), (1,)), ((), ()))


def _dot(a, b):
    return jnp.dot(a, b, preferred_element_type=F32)


def _dot_nt(a, b):
    return lax.dot_general(a, b, NT, preferred_element_type=F32)


def _unpack_heads(w_ref, j, rows):
    w32 = w_ref.bitcast(jnp.uint32)
    u = w32[pl.ds(j, rows, stride=H // 2), :]
    lo = pltpu.bitcast(u << 16, F32).astype(BF16)
    hi = pltpu.bitcast(u & np.uint32(0xFFFF0000), F32).astype(BF16)
    return jnp.concatenate([lo, hi], axis=1)


def _perm(rows, off):
    r = lax.broadcasted_iota(jnp.int32, (rows, MP), 0)
    c = lax.broadcasted_iota(jnp.int32, (rows, MP), 1)
    d = c >> 5
    src = (c & 31) * DH + d + off
    return jnp.where((r == src) & (d < DH), 1.0, 0.0).astype(BF16)


def _kernel(xT_ref, wqkv_ref, awo_ref, gw_ref, c_hbm, wq_hbm, wuk_hbm, wuv_hbm, wo_hbm,
            out_ref,
            x_s, c_s, wq_s, wuk_s, wuv_s, wo_s, ka_s, va_s, oa_s, acc_s, q_s, k_s, v_s, ctx_s, wq2, wk2, wv2, sems):
    copies = [pltpu.make_async_copy(src, dst, sems.at[i]) for i, (src, dst) in enumerate(
        [(c_hbm, c_s), (wq_hbm, wq_s), (wuk_hbm, wuk_s), (wuv_hbm, wuv_s), (wo_hbm, wo_s)])]
    for cp in copies:
        cp.start()

    for t in range(S // 512):
        x_s[t * 512:(t + 1) * 512, :] = xT_ref[:, t * 512:(t + 1) * 512].astype(F32).T.astype(BF16)

    wq_a = _dot(wqkv_ref[:, 0:640], _perm(640, 0)).astype(BF16)
    wk_a = _dot(wqkv_ref[:, 512:1152], _perm(640, 64)).astype(BF16)
    wv_a = _dot(wqkv_ref[:, 1152:1728], _perm(576, 0)).astype(BF16)
    PAD = 16
    ka_s[0:PAD, :] = jnp.zeros((PAD, MP), F32)
    va_s[0:PAD, :] = jnp.zeros((PAD, MP), F32)
    CH = 256
    ri = lax.broadcasted_iota(jnp.int32, (128, 128), 0)
    ci = lax.broadcasted_iota(jnp.int32, (128, 128), 1)
    jm = jnp.where((ri & 31) == (ci & 31), 1.0, 0.0).astype(BF16)
    for t in range(S // CH):
        xs = x_s[t * CH:(t + 1) * CH, :]
        ka_s[PAD + t * CH:PAD + (t + 1) * CH, :] = _dot(xs, wk_a)
        va_s[PAD + t * CH:PAD + (t + 1) * CH, :] = _dot(xs, wv_a)
    for t in range(S // CH):
        xs = x_s[t * CH:(t + 1) * CH, :]
        qa = _dot(xs, wq_a) * (DH ** -0.5 * LOG2E)
        logits = []
        for w in range(W):
            base = PAD + t * CH - DIL * w
            pr = qa * ka_s[base:base + CH, :]
            ps = pr[:, 0:128] + pr[:, 128:256] + pr[:, 256:384] + pr[:, 384:512] + pr[:, 512:640]
            ps = ps + pltpu.roll(ps, 64, 1)
            ps = ps + pltpu.roll(ps, 32, 1)
            if t == 0 and w > 0:
                pos = lax.broadcasted_iota(jnp.int32, (CH, 128), 0)
                ps = jnp.where(pos >= DIL * w, ps, -1e9)
            logits.append(ps)
        mx = functools.reduce(jnp.maximum, logits)
        es = [jnp.exp2(l - mx) for l in logits]
        inv = 1.0 / functools.reduce(lambda a, b: a + b, es)
        o = None
        for w in range(W):
            base = PAD + t * CH - DIL * w
            p = es[w] * inv
            term = jnp.concatenate([p] * 5, axis=1) * va_s[base:base + CH, :]
            o = term if o is None else o + term
        oa_s[t * CH:(t + 1) * CH, :] = o.astype(BF16)
    awoT = _dot(awo_ref[...].astype(F32).T.astype(BF16), _perm(576, 0)).astype(BF16)
    gw = jnp.broadcast_to(gw_ref[...], (16, M))
    for t in range(S // 512):
        sl = slice(t * 512, (t + 1) * 512)
        g = jax.nn.sigmoid(_dot(gw, xT_ref[:, sl])[0:1, :])
        acc_s[:, sl] = g * _dot_nt(awoT, oa_s[sl, :])
    for cp in copies:
        cp.wait()

    for j in range(H // 2):
        wq2[j] = _unpack_heads(wq_s, j, M)
        wk2[j] = _unpack_heads(wuk_s, j, DC)
        wv2[j] = _unpack_heads(wuv_s, j, DC)

    def pair(j, carry):
        wq, wk, wv = wq2[j], wk2[j], wv2[j]
        for t in range(S // 512):
            sl = slice(t * 512, (t + 1) * 512)
            q_s[sl, :] = (_dot(x_s[sl, :], wq) * (D ** -0.5 * LOG2E)).astype(BF16)
            cc = c_s[sl, :]
            k_s[sl, :] = _dot(cc, wk).astype(BF16)
            v_s[sl, :] = _dot(cc, wv).astype(BF16)
        for hh in range(2):
            ls = slice(hh * D, (hh + 1) * D)
            for i in range(S // BQ):
                n = (i + 1) * BQ
                s = _dot_nt(q_s[i * BQ:n, ls], k_s[0:n, ls])
                rr = lax.broadcasted_iota(jnp.int32, (BQ, BQ), 0)
                cc = lax.broadcasted_iota(jnp.int32, (BQ, BQ), 1)
                sd = jnp.where(cc <= rr, s[:, n - BQ:], -1e30)
                s = sd if i == 0 else jnp.concatenate([s[:, :n - BQ], sd], axis=1)
                m = jnp.max(s, axis=1, keepdims=True)
                p = jnp.exp2(s - m)
                l = jnp.sum(p, axis=1, keepdims=True)
                o = _dot(p.astype(BF16), v_s[0:n, ls])
                ctx_s[j, i * BQ:n, ls] = (o / l).astype(BF16)
        return carry

    lax.fori_loop(0, H // 2, pair, 0)

    for t in range(S // 256):
        sl = slice(t * 256, (t + 1) * 256)
        o = None
        for h in range(H):
            term = _dot_nt(wo_s[h * M:(h + 1) * M, :], ctx_s[h // 2, sl, (h % 2) * D:(h % 2 + 1) * D])
            o = term if o is None else o + term
        g = jax.nn.sigmoid(_dot(gw, xT_ref[:, sl])[0:1, :])
        out_ref[:, sl] = (acc_s[0:M, sl] + (1.0 - g) * o).astype(out_ref.dtype)


@jax.jit
def pallas_gated_mix__sliding_local_dilated__compressed_kv_cla__prompt_kernel(
        A_x, A_wqkv, A_wo, B_x, B_c_kv, B_w_q, B_w_uk, B_w_uv, B_w_o, gate_w):
    del B_x
    xT = A_x[0].T
    c = B_c_kv[0]
    wq = B_w_q.reshape(M * H, D)
    wuk = B_w_uk.reshape(DC * H, D)
    wuv = B_w_uv.reshape(DC * H, D)
    woT = B_w_o.transpose(0, 2, 1).reshape(H * M, D)
    gw = gate_w.reshape(1, M)
    vm = pl.BlockSpec(memory_space=pltpu.VMEM)
    hbm = pl.BlockSpec(memory_space=pl.ANY)
    outT = pl.pallas_call(
        _kernel,
        out_shape=jax.ShapeDtypeStruct((M, S), A_x.dtype),
        in_specs=[vm, vm, vm, vm, hbm, hbm, hbm, hbm, hbm],
        out_specs=vm,
        scratch_shapes=[
            pltpu.VMEM((S, M), BF16),
            pltpu.VMEM((S, DC), BF16),
            pltpu.VMEM((M * H, D), BF16),
            pltpu.VMEM((DC * H, D), BF16),
            pltpu.VMEM((DC * H, D), BF16),
            pltpu.VMEM((H * M, D), BF16),
            pltpu.VMEM((S + 16, MP), F32),
            pltpu.VMEM((S + 16, MP), F32),
            pltpu.VMEM((S, MP), BF16),
            pltpu.VMEM((M, S), F32),
            pltpu.VMEM((S, 2 * D), BF16),
            pltpu.VMEM((S, 2 * D), BF16),
            pltpu.VMEM((S, 2 * D), BF16),
            pltpu.VMEM((H // 2, S, 2 * D), BF16),
            pltpu.VMEM((H // 2, M, 2 * D), BF16),
            pltpu.VMEM((H // 2, DC, 2 * D), BF16),
            pltpu.VMEM((H // 2, DC, 2 * D), BF16),
            pltpu.SemaphoreType.DMA((5,)),
        ],
        compiler_params=pltpu.CompilerParams(vmem_limit_bytes=110 * 1024 * 1024),
    )(xT, A_wqkv, A_wo, gw, c, wq, wuk, wuv, woT)
    return outT.T[None]
```

```python
import functools
import numpy as np
import jax
import jax.numpy as jnp
from jax import lax
import jax.experimental.pallas as pl
import jax.experimental.pallas.tpu as pltpu

S = 2048
M = 576
H = 32
D = 128
DC = 512
DH = 18
W = 8
DIL = 2
MP = 640
BQ = 512
T = 128
PM = 2048
PA = 1024
PAD = 16
CH = 256
LOG2E = 1.4426950408889634
F32 = jnp.float32
BF16 = jnp.bfloat16
NT = (((1,), (1,)), ((), ()))


def _dot(a, b):
    return jnp.dot(a, b, preferred_element_type=F32)


def _dot_nt(a, b):
    return lax.dot_general(a, b, NT, preferred_element_type=F32)


def _unpack_heads(w_ref, j, rows):
    w32 = w_ref.bitcast(jnp.uint32)
    u = w32[pl.ds(j, rows, stride=H // 2), :]
    lo = pltpu.bitcast(u << 16, F32).astype(BF16)
    hi = pltpu.bitcast(u & np.uint32(0xFFFF0000), F32).astype(BF16)
    return jnp.concatenate([lo, hi], axis=1)


def _perm(rows, off):
    r = lax.broadcasted_iota(jnp.int32, (rows, MP), 0)
    c = lax.broadcasted_iota(jnp.int32, (rows, MP), 1)
    d = c >> 5
    src = (c & 31) * DH + d + off
    return jnp.where((r == src) & (d < DH), 1.0, 0.0).astype(BF16)


def _kernel(xT_ref, wqkv_ref, awo_ref, gw_ref, c_hbm, wq_hbm, wuk_hbm, wuv_hbm, wo_hbm,
            out_ref,
            x_s, c_s, wo_s, ka_s, va_s, qa_s, q_s, k_s, v_s, ctx_s, wq2, wk2, wv2, sems):
    def prologue(wq_s, wuk_s, wuv_s):
        copies = [pltpu.make_async_copy(src, dst, sems.at[i]) for i, (src, dst) in enumerate(
            [(c_hbm, c_s), (wq_hbm, wq_s), (wuk_hbm, wuk_s), (wuv_hbm, wuv_s), (wo_hbm, wo_s)])]
        for cp in copies:
            cp.start()

        for t in range(S // 512):
            x_s[t * 512:(t + 1) * 512, :] = xT_ref[:, t * 512:(t + 1) * 512].astype(F32).T.astype(BF16)

        wq_a = _dot(wqkv_ref[:, 0:640], _perm(640, 0)).astype(BF16)
        wk_a = _dot(wqkv_ref[:, 512:1152], _perm(640, 64)).astype(BF16)
        wv_a = _dot(wqkv_ref[:, 1152:1728], _perm(576, 0)).astype(BF16)
        ka_s[0:PAD, :] = jnp.zeros((PAD, MP), F32)
        va_s[0:PAD, :] = jnp.zeros((PAD, MP), F32)
        for t in range(S // PA):
            xs = x_s[t * PA:(t + 1) * PA, :]
            qa_s[t * PA:(t + 1) * PA, :] = _dot(xs, wq_a) * (DH ** -0.5 * LOG2E)
        for cp in copies:
            cp.wait()
        for t in range(S // PA):
            xs = x_s[t * PA:(t + 1) * PA, :]
            ka_s[PAD + t * PA:PAD + (t + 1) * PA, :] = _dot(xs, wk_a)
            va_s[PAD + t * PA:PAD + (t + 1) * PA, :] = _dot(xs, wv_a)
            for j in range(t * PA // 128, (t + 1) * PA // 128):
                wq2[j] = _unpack_heads(wq_s, j, M)
                wk2[j] = _unpack_heads(wuk_s, j, DC)
                wv2[j] = _unpack_heads(wuv_s, j, DC)

    pl.run_scoped(prologue, pltpu.VMEM((M * H, D), BF16), pltpu.VMEM((DC * H, D), BF16),
                  pltpu.VMEM((DC * H, D), BF16))

    def attn(j, hh, i):
        ls = slice(hh * D, (hh + 1) * D)
        r0, r1 = i * BQ, (i + 1) * BQ
        G = BQ // T
        tri = lax.broadcasted_iota(jnp.int32, (T, T), 1) <= lax.broadcasted_iota(jnp.int32, (T, T), 0)
        s_off = _dot_nt(q_s[r0:r1, ls], k_s[0:r0, ls]) if i else None
        s_dg = [_dot_nt(q_s[r0 + c * T:r1, ls], k_s[r0 + c * T:r0 + (c + 1) * T, ls]) for c in range(G)]
        ps, inv = [], []
        for g in range(G):
            parts = [s_off[g * T:(g + 1) * T]] if i else []
            parts += [s_dg[c][(g - c) * T:(g - c + 1) * T] for c in range(g)]
            parts.append(jnp.where(tri, s_dg[g][0:T], -1e30))
            sc = jnp.concatenate(parts, axis=1)
            pe = jnp.exp2(sc - jnp.max(sc, axis=1, keepdims=True))
            inv.append(1.0 / jnp.sum(pe, axis=1, keepdims=True))
            ps.append(pe.astype(BF16))
        o_off = _dot(jnp.concatenate([p[:, :r0] for p in ps], axis=0), v_s[0:r0, ls]) if i else None
        o_dg = [_dot(jnp.concatenate([p[:, r0 + c * T:r0 + (c + 1) * T] for p in ps[c:]], axis=0),
                     v_s[r0 + c * T:r0 + (c + 1) * T, ls]) for c in range(G)]
        for g in range(G):
            o = o_off[g * T:(g + 1) * T] if i else None
            for c in range(g + 1):
                term = o_dg[c][(g - c) * T:(g - c + 1) * T]
                o = term if o is None else o + term
            ctx_s[j, r0 + g * T:r0 + (g + 1) * T, ls] = (o * inv[g]).astype(BF16)

    def pair(j, carry):
        for t in range(S // PM):
            sl = slice(t * PM, (t + 1) * PM)
            q_s[sl, :] = (_dot(x_s[sl, :], wq2[j]) * (D ** -0.5 * LOG2E)).astype(BF16)
            kv = _dot(c_s[sl, :], jnp.concatenate([wk2[j], wv2[j]], axis=1)).astype(BF16)
            k_s[sl, :] = kv[:, :2 * D]
            v_s[sl, :] = kv[:, 2 * D:]
        for hh in range(2):
            for i in range(S // BQ):
                attn(j, hh, i)
        return carry

    lax.fori_loop(0, H // 2, pair, 0)

    awoT = _dot(awo_ref[...].astype(F32).T.astype(BF16), _perm(576, 0)).astype(BF16)
    gw = jnp.broadcast_to(gw_ref[...], (16, M))
    for t in range(S // CH):
        sl = slice(t * CH, (t + 1) * CH)
        ob = None
        for h in range(H):
            term = _dot_nt(wo_s[h * M:(h + 1) * M, :], ctx_s[h // 2, sl, (h % 2) * D:(h % 2 + 1) * D])
            ob = term if ob is None else ob + term
        qa = qa_s[sl, :]
        logits = []
        for w in range(W):
            base = PAD + t * CH - DIL * w
            pr = qa * ka_s[base:base + CH, :]
            ps = pr[:, 0:128] + pr[:, 128:256] + pr[:, 256:384] + pr[:, 384:512] + pr[:, 512:640]
            ps = ps + pltpu.roll(ps, 64, 1)
            ps = ps + pltpu.roll(ps, 32, 1)
            if t == 0 and w > 0:
                pos = lax.broadcasted_iota(jnp.int32, (CH, 128), 0)
                ps = jnp.where(pos >= DIL * w, ps, -1e9)
            logits.append(ps)
        mx = functools.reduce(jnp.maximum, logits)
        es = [jnp.exp2(l - mx) for l in logits]
        inv = 1.0 / functools.reduce(lambda a, b: a + b, es)
        o = None
        for w in range(W):
            base = PAD + t * CH - DIL * w
            p = es[w] * inv
            term = jnp.concatenate([p] * 5, axis=1) * va_s[base:base + CH, :]
            o = term if o is None else o + term
        oa = _dot_nt(awoT, o.astype(BF16))
        g = jax.nn.sigmoid(_dot(gw, xT_ref[:, sl])[0:1, :])
        out_ref[:, sl] = (g * oa + (1.0 - g) * ob).astype(out_ref.dtype)


@jax.jit
def pallas_gated_mix__sliding_local_dilated__compressed_kv_cla__prompt_kernel(
        A_x, A_wqkv, A_wo, B_x, B_c_kv, B_w_q, B_w_uk, B_w_uv, B_w_o, gate_w):
    del B_x
    xT = A_x[0].T
    c = B_c_kv[0]
    wq = B_w_q.reshape(M * H, D)
    wuk = B_w_uk.reshape(DC * H, D)
    wuv = B_w_uv.reshape(DC * H, D)
    woT = B_w_o.transpose(0, 2, 1).reshape(H * M, D)
    gw = gate_w.reshape(1, M)
    vm = pl.BlockSpec(memory_space=pltpu.VMEM)
    hbm = pl.BlockSpec(memory_space=pl.ANY)
    outT = pl.pallas_call(
        _kernel,
        out_shape=jax.ShapeDtypeStruct((M, S), A_x.dtype),
        in_specs=[vm, vm, vm, vm, hbm, hbm, hbm, hbm, hbm],
        out_specs=vm,
        scratch_shapes=[
            pltpu.VMEM((S, M), BF16),
            pltpu.VMEM((S, DC), BF16),
            pltpu.VMEM((H * M, D), BF16),
            pltpu.VMEM((S + 16, MP), F32),
            pltpu.VMEM((S + 16, MP), F32),
            pltpu.VMEM((S, MP), F32),
            pltpu.VMEM((S, 2 * D), BF16),
            pltpu.VMEM((S, 2 * D), BF16),
            pltpu.VMEM((S, 2 * D), BF16),
            pltpu.VMEM((H // 2, S, 2 * D), BF16),
            pltpu.VMEM((H // 2, M, 2 * D), BF16),
            pltpu.VMEM((H // 2, DC, 2 * D), BF16),
            pltpu.VMEM((H // 2, DC, 2 * D), BF16),
            pltpu.SemaphoreType.DMA((5,)),
        ],
        compiler_params=pltpu.CompilerParams(vmem_limit_bytes=126 * 1024 * 1024),
    )(xT, A_wqkv, A_wo, gw, c, wq, wuk, wuv, woT)
    return outT.T[None]
```

```python
import functools
import numpy as np
import jax
import jax.numpy as jnp
from jax import lax
import jax.experimental.pallas as pl
import jax.experimental.pallas.tpu as pltpu

S = 2048
M = 576
H = 32
D = 128
DC = 512
DH = 18
W = 8
DIL = 2
MP = 640
BQ = 512
T = 128
PM = 2048
PA = 1024
PAD = 16
CH = 256
LOG2E = 1.4426950408889634
F32 = jnp.float32
BF16 = jnp.bfloat16
NT = (((1,), (1,)), ((), ()))


def _dot(a, b):
    return jnp.dot(a, b, preferred_element_type=F32)


def _dot_nt(a, b):
    return lax.dot_general(a, b, NT, preferred_element_type=F32)


def _unpack_heads(w_ref, j, rows):
    w32 = w_ref.bitcast(jnp.uint32)
    u = w32[pl.ds(j, rows, stride=H // 2), :]
    lo = pltpu.bitcast(u << 16, F32).astype(BF16)
    hi = pltpu.bitcast(u & np.uint32(0xFFFF0000), F32).astype(BF16)
    return jnp.concatenate([lo, hi], axis=1)


def _perm(rows, off):
    r = lax.broadcasted_iota(jnp.int32, (rows, MP), 0)
    c = lax.broadcasted_iota(jnp.int32, (rows, MP), 1)
    d = c >> 5
    src = (c & 31) * DH + d + off
    return jnp.where((r == src) & (d < DH), 1.0, 0.0).astype(BF16)


def _kernel(xT_ref, wqkv_ref, awo_ref, gw_ref, c_hbm, wq_hbm, wuk_hbm, wuv_hbm, wo_hbm,
            out_ref,
            x_s, c_s, wo_s, ka_s, va_s, qa_s, q_s, k_s, v_s, a_s, acc_s, wq2, wk2, wv2, sems):
    def prologue(wq_s, wuk_s, wuv_s):
        copies = [pltpu.make_async_copy(src, dst, sems.at[i]) for i, (src, dst) in enumerate(
            [(c_hbm, c_s), (wq_hbm, wq_s), (wuk_hbm, wuk_s), (wuv_hbm, wuv_s), (wo_hbm, wo_s)])]
        for cp in copies:
            cp.start()

        for t in range(S // 512):
            x_s[t * 512:(t + 1) * 512, :] = xT_ref[:, t * 512:(t + 1) * 512].astype(F32).T.astype(BF16)

        wq_a = _dot(wqkv_ref[:, 0:640], _perm(640, 0)).astype(BF16)
        wk_a = _dot(wqkv_ref[:, 512:1152], _perm(640, 64)).astype(BF16)
        wv_a = _dot(wqkv_ref[:, 1152:1728], _perm(576, 0)).astype(BF16)
        ka_s[0:PAD, :] = jnp.zeros((PAD, MP), F32)
        va_s[0:PAD, :] = jnp.zeros((PAD, MP), F32)
        for t in range(S // PA):
            xs = x_s[t * PA:(t + 1) * PA, :]
            qa_s[t * PA:(t + 1) * PA, :] = _dot(xs, wq_a) * (DH ** -0.5 * LOG2E)
        for t in range(S // PA):
            xs = x_s[t * PA:(t + 1) * PA, :]
            ka_s[PAD + t * PA:PAD + (t + 1) * PA, :] = _dot(xs, wk_a)
            va_s[PAD + t * PA:PAD + (t + 1) * PA, :] = _dot(xs, wv_a)
        awoT = _dot(awo_ref[...].astype(F32).T.astype(BF16), _perm(576, 0)).astype(BF16)
        for t in range(S // CH):
            sl = slice(t * CH, (t + 1) * CH)
            qa = qa_s[sl, :]
            logits = []
            for w in range(W):
                base = PAD + t * CH - DIL * w
                pr = qa * ka_s[base:base + CH, :]
                ps = pr[:, 0:128] + pr[:, 128:256] + pr[:, 256:384] + pr[:, 384:512] + pr[:, 512:640]
                ps = ps + pltpu.roll(ps, 64, 1)
                ps = ps + pltpu.roll(ps, 32, 1)
                if t == 0 and w > 0:
                    pos = lax.broadcasted_iota(jnp.int32, (CH, 128), 0)
                    ps = jnp.where(pos >= DIL * w, ps, -1e9)
                logits.append(ps)
            mx = functools.reduce(jnp.maximum, logits)
            es = [jnp.exp2(l - mx) for l in logits]
            inv = 1.0 / functools.reduce(lambda a, b: a + b, es)
            o = None
            for w in range(W):
                base = PAD + t * CH - DIL * w
                p = es[w] * inv
                term = jnp.concatenate([p] * 5, axis=1) * va_s[base:base + CH, :]
                o = term if o is None else o + term
            a_s[:, sl] = _dot_nt(awoT, o.astype(BF16))
            acc_s[:, sl] = jnp.zeros((M, CH), F32)
        for cp in copies:
            cp.wait()
        for j in range(H // 2):
            wq2[j] = _unpack_heads(wq_s, j, M)
            wk2[j] = _unpack_heads(wuk_s, j, DC)
            wv2[j] = _unpack_heads(wuv_s, j, DC)

    pl.run_scoped(prologue, pltpu.VMEM((M * H, D), BF16), pltpu.VMEM((DC * H, D), BF16),
                  pltpu.VMEM((DC * H, D), BF16))

    def attn(j, hh, i):
        ls = slice(hh * D, (hh + 1) * D)
        r0, r1 = i * BQ, (i + 1) * BQ
        G = BQ // T
        tri = lax.broadcasted_iota(jnp.int32, (T, T), 1) <= lax.broadcasted_iota(jnp.int32, (T, T), 0)
        s_off = _dot_nt(q_s[r0:r1, ls], k_s[0:r0, ls]) if i else None
        s_dg = [_dot_nt(q_s[r0 + c * T:r1, ls], k_s[r0 + c * T:r0 + (c + 1) * T, ls]) for c in range(G)]
        ps, inv = [], []
        for g in range(G):
            parts = [s_off[g * T:(g + 1) * T]] if i else []
            parts += [s_dg[c][(g - c) * T:(g - c + 1) * T] for c in range(g)]
            parts.append(jnp.where(tri, s_dg[g][0:T], -1e30))
            sc = jnp.concatenate(parts, axis=1)
            pe = jnp.exp2(sc - jnp.max(sc, axis=1, keepdims=True))
            inv.append(1.0 / jnp.sum(pe, axis=1, keepdims=True))
            ps.append(pe.astype(BF16))
        o_off = _dot(jnp.concatenate([p[:, :r0] for p in ps], axis=0), v_s[0:r0, ls]) if i else None
        o_dg = [_dot(jnp.concatenate([p[:, r0 + c * T:r0 + (c + 1) * T] for p in ps[c:]], axis=0),
                     v_s[r0 + c * T:r0 + (c + 1) * T, ls]) for c in range(G)]
        ctx = []
        for g in range(G):
            o = o_off[g * T:(g + 1) * T] if i else None
            for c in range(g + 1):
                term = o_dg[c][(g - c) * T:(g - c + 1) * T]
                o = term if o is None else o + term
            ctx.append((o * inv[g]).astype(BF16))
        return jnp.concatenate(ctx, axis=0)

    def pair(j, carry):
        for t in range(S // PM):
            sl = slice(t * PM, (t + 1) * PM)
            q_s[sl, :] = (_dot(x_s[sl, :], wq2[j]) * (D ** -0.5 * LOG2E)).astype(BF16)
            kv = _dot(c_s[sl, :], jnp.concatenate([wk2[j], wv2[j]], axis=1)).astype(BF16)
            k_s[sl, :] = kv[:, :2 * D]
            v_s[sl, :] = kv[:, 2 * D:]
        wo = jnp.concatenate(
            [wo_s[pl.ds(pl.multiple_of((2 * j + hh) * M, M), M), :] for hh in range(2)], axis=1)
        for i in range(S // BQ):
            ctx = jnp.concatenate([attn(j, hh, i) for hh in range(2)], axis=1)
            acc_s[:, i * BQ:(i + 1) * BQ] += _dot_nt(wo, ctx)
        return carry

    lax.fori_loop(0, H // 2, pair, 0)

    gw = jnp.broadcast_to(gw_ref[...], (16, M))
    for t in range(S // 512):
        sl = slice(t * 512, (t + 1) * 512)
        g = jax.nn.sigmoid(_dot(gw, xT_ref[:, sl])[0:1, :])
        out_ref[:, sl] = (g * a_s[:, sl] + (1.0 - g) * acc_s[:, sl]).astype(out_ref.dtype)


@jax.jit
def pallas_gated_mix__sliding_local_dilated__compressed_kv_cla__prompt_kernel(
        A_x, A_wqkv, A_wo, B_x, B_c_kv, B_w_q, B_w_uk, B_w_uv, B_w_o, gate_w):
    del B_x
    xT = A_x[0].T
    c = B_c_kv[0]
    wq = B_w_q.reshape(M * H, D)
    wuk = B_w_uk.reshape(DC * H, D)
    wuv = B_w_uv.reshape(DC * H, D)
    woT = B_w_o.transpose(0, 2, 1).reshape(H * M, D)
    gw = gate_w.reshape(1, M)
    vm = pl.BlockSpec(memory_space=pltpu.VMEM)
    hbm = pl.BlockSpec(memory_space=pl.ANY)
    outT = pl.pallas_call(
        _kernel,
        out_shape=jax.ShapeDtypeStruct((M, S), A_x.dtype),
        in_specs=[vm, vm, vm, vm, hbm, hbm, hbm, hbm, hbm],
        out_specs=vm,
        scratch_shapes=[
            pltpu.VMEM((S, M), BF16),
            pltpu.VMEM((S, DC), BF16),
            pltpu.VMEM((H * M, D), BF16),
            pltpu.VMEM((S + 16, MP), F32),
            pltpu.VMEM((S + 16, MP), F32),
            pltpu.VMEM((S, MP), F32),
            pltpu.VMEM((S, 2 * D), BF16),
            pltpu.VMEM((S, 2 * D), BF16),
            pltpu.VMEM((S, 2 * D), BF16),
            pltpu.VMEM((M, S), F32),
            pltpu.VMEM((M, S), F32),
            pltpu.VMEM((H // 2, M, 2 * D), BF16),
            pltpu.VMEM((H // 2, DC, 2 * D), BF16),
            pltpu.VMEM((H // 2, DC, 2 * D), BF16),
            pltpu.SemaphoreType.DMA((5,)),
        ],
        compiler_params=pltpu.CompilerParams(vmem_limit_bytes=126 * 1024 * 1024),
    )(xT, A_wqkv, A_wo, gw, c, wq, wuk, wuv, woT)
    return outT.T[None]
```

```python
import functools
import numpy as np
import jax
import jax.numpy as jnp
from jax import lax
import jax.experimental.pallas as pl
import jax.experimental.pallas.tpu as pltpu

S = 2048
M = 576
H = 32
D = 128
DC = 512
DH = 18
W = 8
DIL = 2
MP = 640
QB = 2048
PB = 128
OB = 256
T = 128
PM = 2048
PA = 1024
PAD = 16
CH = 128
LOG2E = 1.4426950408889634
F32 = jnp.float32
BF16 = jnp.bfloat16
NT = (((1,), (1,)), ((), ()))


def _dot(a, b):
    return jnp.dot(a, b, preferred_element_type=F32)


def _dot_nt(a, b):
    return lax.dot_general(a, b, NT, preferred_element_type=F32)


def _unpack_heads(u):
    lo = pltpu.bitcast(u << 16, F32).astype(BF16)
    hi = pltpu.bitcast(u & np.uint32(0xFFFF0000), F32).astype(BF16)
    return jnp.concatenate([lo, hi], axis=1)


def _head_minor_rows(t_ref, off, d0, d1):
    return jnp.concatenate(
        [jnp.concatenate([t_ref[n, pl.ds(off + d, H, stride=DH), :] for d in range(d0, d1)], axis=0)
         for n in range(5)], axis=1)[:, :M]


def _kernel(xT_hbm, wqkv_hbm, awo_hbm, gw_ref, c_hbm, wq_hbm, wuk_hbm, wuv_hbm, wo_hbm,
            out_hbm,
            xT_ref, wqkv_ref, awo_ref, out_s, sem_x, sem_o,
            x_s, c_s, wo_s, ka_s, va_s, qa_s, q_s, k_s, v_s, a_s, acc_s, awoT_s, t_s, wq2, wk2, wv2, sems, sem_q, sem_k, sem_v):
    w_copy = pltpu.make_async_copy(wqkv_hbm, wqkv_ref, sems.at[0])
    x_copies = [pltpu.make_async_copy(xT_hbm.at[:, t * PA:(t + 1) * PA], xT_ref.at[:, t * PA:(t + 1) * PA],
                                      sem_x.at[t]) for t in range(S // PA)]
    whole = [pltpu.make_async_copy(src, dst, sems.at[1 + n])
             for n, (src, dst) in enumerate([(awo_hbm, awo_ref), (c_hbm, c_s), (wo_hbm, wo_s)])]
    wsets = [(wq_hbm, wq2, sem_q), (wuk_hbm, wk2, sem_k), (wuv_hbm, wv2, sem_v)]

    def start_gather(j):
        for src, dst, sem in wsets:
            pltpu.make_async_copy(src.bitcast(jnp.uint32).at[:, j, :], dst.at[j], sem.at[j]).start()

    w_copy.start()
    x_copies[0].start()
    acc_s[...] = jnp.zeros((M, S), F32)
    w_copy.wait()
    for cp in x_copies[1:]:
        cp.start()

    for n in range(5):
        rows = min(128, M - n * 128)
        wT = wqkv_ref[n * 128:n * 128 + rows, :].astype(F32)
        if rows < 128:
            wT = jnp.concatenate([wT, jnp.zeros((128 - rows, 3 * M), F32)], axis=0)
        t_s[n] = wT.T
    zero = jnp.zeros((64, M), F32)
    wa = jnp.concatenate(
        [_head_minor_rows(t_s, 0, 0, 16), _head_minor_rows(t_s, M, 0, 16), _head_minor_rows(t_s, 2 * M, 0, DH),
         zero, _head_minor_rows(t_s, 0, 16, DH), _head_minor_rows(t_s, M, 16, DH)], axis=0).astype(BF16)
    ka_s[0:PAD, :] = jnp.zeros((PAD, MP), F32)
    va_s[0:PAD, :] = jnp.zeros((PAD, MP), F32)
    low = lax.broadcasted_iota(jnp.int32, (PA, 128), 1) < 64
    for t in range(S // PA):
        sl = slice(t * PA, (t + 1) * PA)
        pl_ = slice(PAD + t * PA, PAD + (t + 1) * PA)
        x_copies[t].wait()
        if t == 0:
            for cp in whole:
                cp.start()
            start_gather(0)
        xs = xT_ref[:, sl].T
        x_s[sl, :] = xs
        r = _dot_nt(xs, wa)
        qa_s[sl, 0:512] = r[:, 0:512] * (DH ** -0.5 * LOG2E)
        ka_s[pl_, 0:512] = r[:, 512:1024]
        va_s[pl_, :] = r[:, 1024:1664]
        rem = r[:, 1664:1792]
        qa_s[sl, 512:640] = jnp.where(low, rem, 0.0) * (DH ** -0.5 * LOG2E)
        ka_s[pl_, 512:640] = jnp.where(low, pltpu.roll(rem, 64, 1), 0.0)
    for cp in whole:
        cp.wait()
    awo = jnp.concatenate([awo_ref[...].astype(F32), jnp.zeros((M, MP - M), F32)], axis=1)
    for n in range(5):
        t_s[n, 0:M, :] = awo[:, n * 128:(n + 1) * 128]
    awoT_s[...] = jnp.concatenate([_head_minor_rows(t_s, 0, 0, DH), zero], axis=0).T.astype(BF16)

    def window(j):
        r = pl.multiple_of(j * CH, CH)
        qa = qa_s[pl.ds(r, CH), :]
        kw = ka_s.at[pl.ds(r, CH + PAD)]
        vw = va_s.at[pl.ds(r, CH + PAD)]
        pos = lax.broadcasted_iota(jnp.int32, (PAD, 128), 0) + r
        logits = []
        for w in range(W):
            base = PAD - DIL * w
            pr = qa * kw[base:base + CH, :]
            ps = pr[:, 0:128] + pr[:, 128:256] + pr[:, 256:384] + pr[:, 384:512] + pr[:, 512:640]
            ps = ps + pltpu.roll(ps, 64, 1)
            ps = ps + pltpu.roll(ps, 32, 1)
            if w > 0:
                ps = jnp.concatenate([jnp.where(pos >= DIL * w, ps[:PAD], -1e30), ps[PAD:]], axis=0)
            logits.append(ps)
        mx = functools.reduce(jnp.maximum, logits)
        es = [jnp.exp2(l - mx) for l in logits]
        inv = 1.0 / functools.reduce(lambda a, b: a + b, es)
        o = None
        for w in range(W):
            base = PAD - DIL * w
            term = jnp.concatenate([es[w] * inv] * 5, axis=1) * vw[base:base + CH, :]
            o = term if o is None else o + term
        o = o.astype(BF16)
        slot = pl.multiple_of(S + (j % 2) * (5 * CH), CH)
        for n in range(5):
            q_s[pl.ds(slot + n * CH, CH), 0:128] = o[:, n * 128:(n + 1) * 128]
        o = jnp.concatenate([q_s[pl.ds(slot + n * CH, CH), 0:128] for n in range(5)], axis=1)
        a_s[j] = _dot_nt(awoT_s[...], o)

    def attn(hh):
        ls = slice(hh * D, (hh + 1) * D)
        tri = lax.broadcasted_iota(jnp.int32, (T, T), 1) <= lax.broadcasted_iota(jnp.int32, (T, T), 0)
        ps, inv = [], []
        for r0 in range(0, S, QB):
            r1 = r0 + QB
            s_off = _dot_nt(q_s[r0:r1, ls], k_s[0:r0, ls]) if r0 else None
            s_dg = [_dot_nt(q_s[r0 + c * T:r1, ls], k_s[r0 + c * T:r0 + (c + 1) * T, ls]) for c in range(QB // T)]
            for g in range(QB // T):
                parts = [s_off[g * T:(g + 1) * T]] if r0 else []
                parts += [s_dg[c][(g - c) * T:(g - c + 1) * T] for c in range(g)]
                parts.append(jnp.where(tri, s_dg[g][0:T], -1e30))
                sc = jnp.concatenate(parts, axis=1)
                pe = jnp.exp2(sc - jnp.max(sc, axis=1, keepdims=True))
                inv.append(1.0 / jnp.sum(pe, axis=1, keepdims=True))
                ps.append(pe.astype(BF16))
        ctx = []
        for r0 in range(0, S, PB):
            pb = ps[r0 // T:(r0 + PB) // T]
            o_off = _dot(jnp.concatenate([p[:, :r0 + T] for p in pb], axis=0), v_s[0:r0 + T, ls])
            o_dg = {c: _dot(jnp.concatenate([p[:, r0 + c * T:r0 + (c + 1) * T] for p in pb[c:]], axis=0),
                            v_s[r0 + c * T:r0 + (c + 1) * T, ls]) for c in range(1, PB // T)}
            for g in range(PB // T):
                o = o_off[g * T:(g + 1) * T]
                for c in range(1, g + 1):
                    o = o + o_dg[c][(g - c) * T:(g - c + 1) * T]
                ctx.append((o * inv[r0 // T + g]).astype(BF16))
        return ctx

    def pair(j, carry):
        pl.when(j + 1 < H // 2)(lambda: start_gather(j + 1))
        for _, dst, sem in wsets:
            pltpu.make_async_copy(dst.at[j], dst.at[j], sem.at[j]).wait()
        for t in range(S // PM):
            sl = slice(t * PM, (t + 1) * PM)
            q_s[sl, :] = (_dot(x_s[sl, :], _unpack_heads(wq2[j])) * (D ** -0.5 * LOG2E)).astype(BF16)
            kv = _dot(c_s[sl, :], jnp.concatenate([_unpack_heads(wk2[j]), _unpack_heads(wv2[j])], axis=1)).astype(BF16)
            k_s[sl, :] = kv[:, :2 * D]
            v_s[sl, :] = kv[:, 2 * D:]
        window(j)
        wo = jnp.concatenate(
            [wo_s[pl.ds(pl.multiple_of((2 * j + hh) * M, M), M), :] for hh in range(2)], axis=1)
        ctx = [attn(hh) for hh in range(2)]
        for r0 in range(0, S, OB):
            blk = jnp.concatenate(
                [jnp.concatenate(c[r0 // T:(r0 + OB) // T], axis=0) for c in ctx], axis=1)
            acc_s[:, r0:r0 + OB] += _dot_nt(wo, blk)
        return carry

    lax.fori_loop(0, H // 2, pair, 0)

    o_copies = [pltpu.make_async_copy(out_s.at[:, t * 512:(t + 1) * 512], out_hbm.at[:, t * 512:(t + 1) * 512],
                                      sem_o.at[t]) for t in range(S // 512)]
    gw = jnp.broadcast_to(gw_ref[...], (16, M))
    for t in range(S // 512):
        sl = slice(t * 512, (t + 1) * 512)
        g = jax.nn.sigmoid(_dot(gw, xT_ref[:, sl])[0:1, :])
        out_s[:, sl] = (g * jnp.concatenate([a_s[4 * t + n] for n in range(4)], axis=1) + (1.0 - g) * acc_s[:, sl]).astype(out_s.dtype)
        o_copies[t].start()
    for cp in o_copies:
        cp.wait()


@jax.jit
def pallas_gated_mix__sliding_local_dilated__compressed_kv_cla__prompt_kernel(
        A_x, A_wqkv, A_wo, B_x, B_c_kv, B_w_q, B_w_uk, B_w_uv, B_w_o, gate_w):
    del B_x
    xT = A_x[0].T
    c = B_c_kv[0]
    wq = B_w_q
    wuk = B_w_uk
    wuv = B_w_uv
    woT = B_w_o.transpose(0, 2, 1).reshape(H * M, D)
    gw = gate_w.reshape(1, M)
    vm = pl.BlockSpec(memory_space=pltpu.VMEM)
    hbm = pl.BlockSpec(memory_space=pl.ANY)
    outT = pl.pallas_call(
        _kernel,
        out_shape=jax.ShapeDtypeStruct((M, S), A_x.dtype),
        in_specs=[hbm, hbm, hbm, vm, hbm, hbm, hbm, hbm, hbm],
        out_specs=hbm,
        scratch_shapes=[
            pltpu.VMEM((M, S), BF16),
            pltpu.VMEM((M, 3 * M), BF16),
            pltpu.VMEM((M, M), BF16),
            pltpu.VMEM((M, S), A_x.dtype),
            pltpu.SemaphoreType.DMA((S // PA,)),
            pltpu.SemaphoreType.DMA((S // 512,)),
            pltpu.VMEM((S, M), BF16),
            pltpu.VMEM((S, DC), BF16),
            pltpu.VMEM((H * M, D), BF16),
            pltpu.VMEM((S + 16, MP), F32),
            pltpu.VMEM((S + 16, MP), F32),
            pltpu.VMEM((S, MP), F32),
            pltpu.VMEM((S + 10 * CH, 2 * D), BF16),
            pltpu.VMEM((S, 2 * D), BF16),
            pltpu.VMEM((S, 2 * D), BF16),
            pltpu.VMEM((S // CH, M, CH), F32),
            pltpu.VMEM((M, S), F32),
            pltpu.VMEM((M, MP), BF16),
            pltpu.VMEM((5, 3 * M, 128), F32),
            pltpu.VMEM((H // 2, M, D), jnp.uint32),
            pltpu.VMEM((H // 2, DC, D), jnp.uint32),
            pltpu.VMEM((H // 2, DC, D), jnp.uint32),
            pltpu.SemaphoreType.DMA((4,)),
            pltpu.SemaphoreType.DMA((H // 2,)),
            pltpu.SemaphoreType.DMA((H // 2,)),
            pltpu.SemaphoreType.DMA((H // 2,)),

        ],
        compiler_params=pltpu.CompilerParams(vmem_limit_bytes=126 * 1024 * 1024),
    )(xT, A_wqkv, A_wo, gw, c, wq, wuk, wuv, woT)
    return outT.T[None]
```

```python
import functools
import numpy as np
import jax
import jax.numpy as jnp
from jax import lax
import jax.experimental.pallas as pl
import jax.experimental.pallas.tpu as pltpu

S = 2048
M = 576
H = 32
D = 128
DC = 512
DH = 18
W = 8
DIL = 2
MP = 640
OB = 256
T = 128
PM = 256
AHEAD = 256
LAG = 2
OLAG = 4
WAT = 4
PA = 1024
PAD = 16
CH = S // (H // 2)
LOG2E = 1.4426950408889634
F32 = jnp.float32
BF16 = jnp.bfloat16
NT = (((1,), (1,)), ((), ()))


def _dot(a, b):
    return jnp.dot(a, b, preferred_element_type=F32)


def _dot_nt(a, b):
    return lax.dot_general(a, b, NT, preferred_element_type=F32)


def _unpack_heads(u):
    lo = pltpu.bitcast(u << 16, F32).astype(BF16)
    hi = pltpu.bitcast(u & np.uint32(0xFFFF0000), F32).astype(BF16)
    return jnp.concatenate([lo, hi], axis=1)


def _head_minor_rows(t_ref, off, d0, d1):
    return jnp.concatenate(
        [jnp.concatenate([t_ref[n, pl.ds(off + d, H, stride=DH), :] for d in range(d0, d1)], axis=0)
         for n in range(5)], axis=1)[:, :M]


def _kernel(xT_hbm, wqkv_hbm, awo_hbm, gw_ref, c_hbm, wq_hbm, wuk_hbm, wuv_hbm, wo_hbm,
            out_hbm,
            xT_ref, wqkv_ref, awo_ref, out_s, sem_x, sem_o,
            x_s, c_s, wo_s, ka_s, va_s, qa_s, q_s, k_s, v_s, a_s, acc_s, awoT_s, t_s, wq2, wk2, wv2, sems, sem_q, sem_k, sem_v):
    w_copy = pltpu.make_async_copy(wqkv_hbm, wqkv_ref, sems.at[0])
    x_copies = [pltpu.make_async_copy(xT_hbm.at[:, t * PA:(t + 1) * PA], xT_ref.at[:, t * PA:(t + 1) * PA],
                                      sem_x.at[t]) for t in range(S // PA)]
    whole = [pltpu.make_async_copy(src, dst, sems.at[1 + n])
             for n, (src, dst) in enumerate([(awo_hbm, awo_ref), (c_hbm, c_s), (wo_hbm, wo_s)])]
    wsets = [(wq_hbm, wq2, sem_q), (wuk_hbm, wk2, sem_k), (wuv_hbm, wv2, sem_v)]

    def start_gather(j):
        for src, dst, sem in wsets:
            pltpu.make_async_copy(src.bitcast(jnp.uint32).at[:, j, :], dst.at[j], sem.at[j]).start()

    w_copy.start()
    x_copies[0].start()
    acc_s[...] = jnp.zeros((M, S), F32)
    w_copy.wait()
    for cp in x_copies[1:]:
        cp.start()

    for n in range(5):
        rows = min(128, M - n * 128)
        wT = wqkv_ref[n * 128:n * 128 + rows, :].astype(F32)
        if rows < 128:
            wT = jnp.concatenate([wT, jnp.zeros((128 - rows, 3 * M), F32)], axis=0)
        t_s[n] = wT.T
    zero = jnp.zeros((64, M), F32)
    wa = jnp.concatenate(
        [_head_minor_rows(t_s, 0, 0, 16), _head_minor_rows(t_s, M, 0, 16), _head_minor_rows(t_s, 2 * M, 0, DH),
         zero, _head_minor_rows(t_s, 0, 16, DH), _head_minor_rows(t_s, M, 16, DH)], axis=0).astype(BF16)
    ka_s[0:PAD, :] = jnp.zeros((PAD, MP), F32)
    va_s[0:PAD, :] = jnp.zeros((PAD, MP), F32)
    low = lax.broadcasted_iota(jnp.int32, (PA, 128), 1) < 64
    for t in range(S // PA):
        sl = slice(t * PA, (t + 1) * PA)
        pl_ = slice(PAD + t * PA, PAD + (t + 1) * PA)
        x_copies[t].wait()
        if t == 0:
            for cp in whole:
                cp.start()
            start_gather(0)
        xs = xT_ref[:, sl].T
        x_s[sl, :] = xs
        r = _dot_nt(xs, wa)
        qa_s[sl, 0:512] = r[:, 0:512] * (DH ** -0.5 * LOG2E)
        ka_s[pl_, 0:512] = r[:, 512:1024]
        va_s[pl_, :] = r[:, 1024:1664]
        rem = r[:, 1664:1792]
        qa_s[sl, 512:640] = jnp.where(low, rem, 0.0) * (DH ** -0.5 * LOG2E)
        ka_s[pl_, 512:640] = jnp.where(low, pltpu.roll(rem, 64, 1), 0.0)
    for cp in whole:
        cp.wait()
    awo = jnp.concatenate([awo_ref[...].astype(F32), jnp.zeros((M, MP - M), F32)], axis=1)
    for n in range(5):
        t_s[n, 0:M, :] = awo[:, n * 128:(n + 1) * 128]
    awoT_s[...] = jnp.concatenate([_head_minor_rows(t_s, 0, 0, DH), zero], axis=0).T.astype(BF16)

    def window(j):
        r = pl.multiple_of(j * CH, CH)
        qa = qa_s[pl.ds(r, CH), :]
        kw = ka_s.at[pl.ds(r, CH + PAD)]
        vw = va_s.at[pl.ds(r, CH + PAD)]
        pos = lax.broadcasted_iota(jnp.int32, (PAD, 128), 0) + r
        logits = []
        for w in range(W):
            base = PAD - DIL * w
            pr = qa * kw[base:base + CH, :]
            ps = pr[:, 0:128] + pr[:, 128:256] + pr[:, 256:384] + pr[:, 384:512] + pr[:, 512:640]
            ps = ps + pltpu.roll(ps, 64, 1)
            ps = ps + pltpu.roll(ps, 32, 1)
            if w > 0:
                ps = jnp.concatenate([jnp.where(pos >= DIL * w, ps[:PAD], -1e30), ps[PAD:]], axis=0)
            logits.append(ps)
        mx = functools.reduce(jnp.maximum, logits)
        es = [jnp.exp2(l - mx) for l in logits]
        inv = 1.0 / functools.reduce(lambda a, b: a + b, es)
        o = None
        for w in range(W):
            base = PAD - DIL * w
            term = jnp.concatenate([es[w] * inv] * 5, axis=1) * vw[base:base + CH, :]
            o = term if o is None else o + term
        a_s[j] = _dot_nt(awoT_s[...], o.astype(BF16))

    def probs(hh, g):
        ls = slice(hh * D, (hh + 1) * D)
        n = (g + 1) * T
        tri = lax.broadcasted_iota(jnp.int32, (T, T), 1) <= lax.broadcasted_iota(jnp.int32, (T, T), 0)
        sc = _dot_nt(q_s[n - T:n, ls], k_s[0:n, ls])
        diag = jnp.where(tri, sc[:, n - T:], -1e30)
        sc = jnp.concatenate([sc[:, :n - T], diag], axis=1) if g else diag
        pe = jnp.exp2(sc - jnp.max(sc, axis=1, keepdims=True))
        return pe.astype(BF16), 1.0 / jnp.sum(pe, axis=1, keepdims=True)

    def context(hh, g, p, inv):
        return (_dot(p, v_s[0:(g + 1) * T, hh * D:(hh + 1) * D]) * inv).astype(BF16)

    def pair(j, carry):
        pl.when(j + 1 < H // 2)(lambda: start_gather(j + 1))
        for _, dst, sem in wsets:
            pltpu.make_async_copy(dst.at[j], dst.at[j], sem.at[j]).wait()
        wq = _unpack_heads(wq2[j])
        wkv = jnp.concatenate([_unpack_heads(wk2[j]), _unpack_heads(wv2[j])], axis=1)
        wo = jnp.concatenate(
            [wo_s[pl.ds(pl.multiple_of((2 * j + hh) * M, M), M), :] for hh in range(2)], axis=1)
        G = S // T
        p, ctx = {}, {}
        done = 0
        items = [(hh, g) for g in range(G) for hh in range(2)]
        for u in range(len(items) + LAG + OLAG):
            while done < S and done < (u // 2 + 1) * T + AHEAD:
                sl = slice(done, done + PM)
                kv = _dot(c_s[sl, :], wkv).astype(BF16)
                k_s[sl, :] = kv[:, :2 * D]
                v_s[sl, :] = kv[:, 2 * D:]
                q_s[sl, :] = (_dot(x_s[sl, :], wq) * (D ** -0.5 * LOG2E)).astype(BF16)
                done += PM
            if u == WAT:
                window(j)
            if u < len(items):
                p[items[u]] = probs(*items[u])
            if 0 <= u - LAG < len(items):
                it = items[u - LAG]
                ctx[it] = context(*it, *p.pop(it))
            e = u - LAG - OLAG + 1
            if e > 0 and e % (2 * OB // T) == 0:
                g1 = e // 2
                g0 = g1 - OB // T
                blk = jnp.concatenate(
                    [jnp.concatenate([ctx.pop((hh, g)) for g in range(g0, g1)], axis=0) for hh in range(2)], axis=1)
                acc_s[:, g0 * T:g1 * T] += _dot_nt(wo, blk)
        return carry

    lax.fori_loop(0, H // 2, pair, 0)

    o_copies = [pltpu.make_async_copy(out_s.at[:, t * 512:(t + 1) * 512], out_hbm.at[:, t * 512:(t + 1) * 512],
                                      sem_o.at[t]) for t in range(S // 512)]
    gw = jnp.broadcast_to(gw_ref[...], (16, M))
    for t in range(S // 512):
        sl = slice(t * 512, (t + 1) * 512)
        g = jax.nn.sigmoid(_dot(gw, xT_ref[:, sl])[0:1, :])
        out_s[:, sl] = (g * jnp.concatenate([a_s[4 * t + n] for n in range(4)], axis=1) + (1.0 - g) * acc_s[:, sl]).astype(out_s.dtype)
        o_copies[t].start()
    for cp in o_copies:
        cp.wait()


@jax.jit
def pallas_gated_mix__sliding_local_dilated__compressed_kv_cla__prompt_kernel(
        A_x, A_wqkv, A_wo, B_x, B_c_kv, B_w_q, B_w_uk, B_w_uv, B_w_o, gate_w):
    del B_x
    xT = A_x[0].T
    c = B_c_kv[0]
    wq = B_w_q
    wuk = B_w_uk
    wuv = B_w_uv
    woT = B_w_o.transpose(0, 2, 1).reshape(H * M, D)
    gw = gate_w.reshape(1, M)
    vm = pl.BlockSpec(memory_space=pltpu.VMEM)
    hbm = pl.BlockSpec(memory_space=pl.ANY)
    outT = pl.pallas_call(
        _kernel,
        out_shape=jax.ShapeDtypeStruct((M, S), A_x.dtype),
        in_specs=[hbm, hbm, hbm, vm, hbm, hbm, hbm, hbm, hbm],
        out_specs=hbm,
        scratch_shapes=[
            pltpu.VMEM((M, S), BF16),
            pltpu.VMEM((M, 3 * M), BF16),
            pltpu.VMEM((M, M), BF16),
            pltpu.VMEM((M, S), A_x.dtype),
            pltpu.SemaphoreType.DMA((S // PA,)),
            pltpu.SemaphoreType.DMA((S // 512,)),
            pltpu.VMEM((S, M), BF16),
            pltpu.VMEM((S, DC), BF16),
            pltpu.VMEM((H * M, D), BF16),
            pltpu.VMEM((S + 16, MP), F32),
            pltpu.VMEM((S + 16, MP), F32),
            pltpu.VMEM((S, MP), F32),
            pltpu.VMEM((S, 2 * D), BF16),
            pltpu.VMEM((S, 2 * D), BF16),
            pltpu.VMEM((S, 2 * D), BF16),
            pltpu.VMEM((S // CH, M, CH), F32),
            pltpu.VMEM((M, S), F32),
            pltpu.VMEM((M, MP), BF16),
            pltpu.VMEM((5, 3 * M, 128), F32),
            pltpu.VMEM((H // 2, M, D), jnp.uint32),
            pltpu.VMEM((H // 2, DC, D), jnp.uint32),
            pltpu.VMEM((H // 2, DC, D), jnp.uint32),
            pltpu.SemaphoreType.DMA((4,)),
            pltpu.SemaphoreType.DMA((H // 2,)),
            pltpu.SemaphoreType.DMA((H // 2,)),
            pltpu.SemaphoreType.DMA((H // 2,)),

        ],
        compiler_params=pltpu.CompilerParams(vmem_limit_bytes=126 * 1024 * 1024),
    )(xT, A_wqkv, A_wo, gw, c, wq, wuk, wuv, woT)
    return outT.T[None]
```
